```python
import os as _os
_os.environ.setdefault("JAX_PLATFORMS", "cpu")
import jax
import jax.numpy as jnp

def _softmax(x, axis=-1):
    return jax.nn.softmax(x, axis=axis)
def _gelu(x):
    return jax.nn.gelu(x, approximate=True)
def _silu(x):
    return jax.nn.silu(x)
def _sigmoid(x):
    return jax.nn.sigmoid(x)
def _layernorm(x, axis=-1, eps=1e-5):
    m = jnp.mean(x, axis=axis, keepdims=True)
    v = jnp.var(x, axis=axis, keepdims=True)
    return (x - m) / jnp.sqrt(v + eps)
def _scatter_add(tgt, idx, src, axis=0):
    return tgt.at[idx].add(src)
def _segment_sum(src, seg, n):
    return jax.ops.segment_sum(src, seg, n)
class _Rng:
    def __init__(self, key):
        self._k = key
    def _next(self):
        self._k, sub = jax.random.split(self._k)
        return sub
    def normal(self, shape):
        return jax.random.normal(self._next(), shape, dtype=jnp.bfloat16)
    def randint(self, lo, hi, shape):
        return jax.random.randint(self._next(), shape, lo, hi, dtype=jnp.int32)
    def uniform(self, shape, lo=0.0, hi=1.0):
        return jax.random.uniform(self._next(), shape, jnp.bfloat16, lo, hi)
    def permutation(self, n):
        return jax.random.permutation(self._next(), n)


kernel_name = 'standalone__se_block__vision'

def setup_inputs():
    _rng = _Rng(jax.random.key(int.from_bytes(__import__("os").urandom(4), "little")))
    _w = (lambda a: (lambda t: t.astype(jnp.bfloat16) if jnp.issubdtype(t.dtype, jnp.floating) else t)(jnp.asarray(a)))
    H = W = 384
    C = 192; r = max(C // 16, 4)
    return {
        "x": _w((lambda *s: _rng.normal(s) * 0.8)(1, H, W, C)),
        "w_down": _w((lambda *s: _rng.normal(s) * 0.8)(C, r)),
        "w_up": _w((lambda *s: _rng.normal(s) * 0.8)(r, C)),
    }

def reference(x, w_down, w_up):
    s = x.mean(axis=(1, 2))
    s = _sigmoid(_silu(s @ w_down) @ w_up)
    return x * s[:, None, None, :]
```

```python
import jax
import jax.numpy as jnp
from jax import lax
import jax.experimental.pallas as pl
import jax.experimental.pallas.tpu as pltpu

_STREAMS = 6
_CC = 48
_LANES = 128


def _read_chunks(streams, rows):
    chunks = [(a, 0, rows) for a in range(streams - 1)]
    start, size = 0, rows // 2
    while size >= 1:
        chunks.append((streams - 1, start, size))
        start += size
        size //= 2
    chunks.append((streams - 1, start, rows - start))
    return chunks


def _se_kernel(x_hbm, wdt_hbm, wu_hbm, o_hbm, buf, wdt_v, wu_v, wut_v, s_v, sems):
    streams, rows, c, w = buf.shape
    chunks = _read_chunks(streams, rows)
    n_lane_blocks = w // _LANES
    w_sem = len(chunks)

    def read(i):
        a, h0, nh = chunks[i]
        return pltpu.make_async_copy(
            x_hbm.at[a, pl.ds(h0, nh)], buf.at[a, pl.ds(h0, nh)], sems.at[i])

    wdt_copy = pltpu.make_async_copy(wdt_hbm, wdt_v, sems.at[w_sem])
    wu_copy = pltpu.make_async_copy(wu_hbm, wu_v, sems.at[w_sem])

    read(0).start()
    wdt_copy.start()
    wu_copy.start()
    for i in range(1, len(chunks)):
        read(i).start()

    wdt_copy.wait()
    wu_copy.wait()
    wut_v[...] = wu_v[...].astype(jnp.float32).T

    acc = jnp.zeros((c, _LANES), jnp.float32)
    for i, (a, h0, nh) in enumerate(chunks):
        read(i).wait()

        def row_sum(h, acc, a=a):
            xf = buf[a, h].astype(jnp.float32)
            part = xf[:, 0:_LANES]
            for j in range(1, n_lane_blocks):
                part = part + xf[:, j * _LANES:(j + 1) * _LANES]
            return acc + part

        acc = lax.fori_loop(h0, h0 + nh, row_sum, acc)

    mean = jnp.sum(acc, axis=1, keepdims=True) * (1.0 / (streams * rows * w))
    mean = jnp.broadcast_to(mean, (c, _LANES)).astype(jnp.bfloat16)
    hid = jnp.dot(wdt_v[...], mean, preferred_element_type=jnp.float32)
    hid = hid.astype(jnp.bfloat16).astype(jnp.float32)
    hid = (hid * jax.nn.sigmoid(hid)).astype(jnp.bfloat16)
    up = jnp.dot(wut_v[...].astype(jnp.bfloat16), hid,
                 preferred_element_type=jnp.float32)
    up = up.astype(jnp.bfloat16).astype(jnp.float32)
    s_v[...] = jax.nn.sigmoid(up).astype(jnp.bfloat16).astype(jnp.float32)

    def write_row(h, carry):
        for c0 in range(0, c, _CC):
            s = s_v[c0:c0 + _CC, :]
            s = jnp.concatenate([s] * n_lane_blocks, axis=1)
            for a in range(streams):
                xf = buf[a, h, c0:c0 + _CC, :].astype(jnp.float32)
                buf[a, h, c0:c0 + _CC, :] = (xf * s).astype(buf.dtype)
            pltpu.make_async_copy(
                buf.at[:, h, pl.ds(c0, _CC), :],
                o_hbm.at[:, h, pl.ds(c0, _CC), :],
                sems.at[0]).start()
        return carry

    lax.fori_loop(0, rows, write_row, 0)
    pltpu.make_async_copy(buf, o_hbm, sems.at[0]).wait()


@jax.jit
def pallas_standalone__se_block__vision_kernel(
    x: jax.Array,
    w_down: jax.Array,
    w_up: jax.Array,
):
    b, hh, ww, c = x.shape
    assert b == 1
    r = w_down.shape[1]
    rows = hh // _STREAMS
    xt = x.transpose(0, 1, 3, 2).reshape(_STREAMS, rows, c, ww)
    n_sems = len(_read_chunks(_STREAMS, rows)) + 1
    out = pl.pallas_call(
        _se_kernel,
        out_shape=jax.ShapeDtypeStruct(xt.shape, x.dtype),
        in_specs=[pl.BlockSpec(memory_space=pl.ANY)] * 3,
        out_specs=pl.BlockSpec(memory_space=pl.ANY),
        scratch_shapes=[
            pltpu.VMEM(xt.shape, x.dtype),
            pltpu.VMEM((r, c), w_down.dtype),
            pltpu.VMEM((r, c), w_up.dtype),
            pltpu.VMEM((c, r), jnp.float32),
            pltpu.VMEM((c, _LANES), jnp.float32),
            pltpu.SemaphoreType.DMA((n_sems,)),
        ],
        compiler_params=pltpu.CompilerParams(vmem_limit_bytes=100 * 1024 * 1024),
    )(xt, w_down.T, w_up)
    return out.reshape(b, hh, c, ww).transpose(0, 1, 3, 2)
```

```python
import jax
import jax.numpy as jnp
from jax import lax
import jax.experimental.pallas as pl
import jax.experimental.pallas.tpu as pltpu

_LANES = 128
_SUB = 8
_STREAMS = 6
_PIECE = 64
_BLOCK = 64
_N_LAST = 2
_FULL = (252, 80, 28)
_HEAD = (14, 6, 3, 1)
_LAST = (16, 5, 2, 1)
_N_READ = len(_FULL) + len(_HEAD) + len(_LAST)
_F32 = jnp.float32
_BF16 = jnp.bfloat16


def _split(start, sizes):
    out = []
    for size in sizes:
        out.append((start, size))
        start += size
    return out


def _tree_sum(vals):
    vals = list(vals)
    while len(vals) > 1:
        nxt = [vals[i] + vals[i + 1] for i in range(0, len(vals) - 1, 2)]
        if len(vals) % 2:
            nxt.append(vals[-1])
        vals = nxt
    return vals[0]


def _round_bf16(v):
    return v.astype(_BF16).astype(_F32)


def _se_kernel(x_hbm, wdt_hbm, wu_hbm, o_hbm,
               buf, wdt_v, wu_v, wdb_v, wub_v, hid_v, s_v, sems):
    hh, rpr, _ = x_hbm.shape
    groups, streams, block, piece, _ = buf.shape
    r, c = wdt_v.shape
    n_cg = c // _SUB
    n_head = n_cg - _N_LAST
    c_head = n_head * _SUB
    n_wb = rpr // c
    grp_rows = n_wb * _SUB
    head_rows = n_head * grp_rows
    phases = rpr // piece
    tpp = piece // _SUB
    gpp = n_cg // (phases - 1)
    inv_n = 1.0 / (hh * n_wb * _LANES)
    n_full = sum(_FULL)
    assert n_full + sum(_HEAD) == hh and n_full + sum(_LAST) == hh
    assert gpp * (phases - 1) == n_cg and gpp * n_wb >= tpp
    full_chunks = _split(0, _FULL)
    head_chunks = _split(n_full, _HEAD)
    last_chunks = _split(n_full, _LAST)
    rows_v = buf.reshape(hh, rpr, _LANES)

    windows = [(pl.ds(h0, nh),) for h0, nh in full_chunks]
    windows += [(pl.ds(h0, nh), pl.ds(0, head_rows)) for h0, nh in head_chunks]
    windows += [(pl.ds(h0, nh), pl.ds(head_rows, rpr - head_rows))
                for h0, nh in last_chunks]
    reads = [pltpu.make_async_copy(x_hbm.at[w], rows_v.at[w], sems.at[i])
             for i, w in enumerate(windows)]
    wdt_copy = pltpu.make_async_copy(wdt_hbm, wdt_v, sems.at[_N_READ])
    wu_copy = pltpu.make_async_copy(wu_hbm, wu_v, sems.at[_N_READ])

    reads[0].start()
    wdt_copy.start()
    wu_copy.start()
    for copy in reads[1:]:
        copy.start()

    wdt_copy.wait()
    wu_copy.wait()
    wdt = wdt_v[...].astype(_F32)
    for k in range(c - c_head):
        wdb_v[k] = jnp.broadcast_to(wdt[:, c_head + k:c_head + k + 1], (r, _LANES))
    wut = wu_v[...].astype(_F32).T * 0.5
    for j in range(r):
        col = jnp.broadcast_to(wut[:, j:j + 1], (c, _LANES))
        wub_v[:, j] = col.reshape(n_cg, _SUB, _LANES)

    def row_sum(n_groups):
        def body(h, acc):
            xf = rows_v[h, 0:n_groups * grp_rows, :].astype(_F32)
            xf = xf.reshape(n_groups, n_wb, _SUB, _LANES)
            part = xf[:, 0]
            for j in range(1, n_wb):
                part = part + xf[:, j]
            return acc + part
        return body

    pending = iter(reads)
    acc = jnp.zeros((n_cg, _SUB, _LANES), _F32)
    for h0, nh in full_chunks:
        next(pending).wait()
        acc = lax.fori_loop(h0, h0 + nh, row_sum(n_cg), acc)
    acc_last = [acc[g] for g in range(n_head, n_cg)]
    acc = acc[:n_head]
    for h0, nh in head_chunks:
        next(pending).wait()
        acc = lax.fori_loop(h0, h0 + nh, row_sum(n_head), acc)

    mean = jnp.sum(acc.reshape(c_head, _LANES), axis=1, keepdims=True) * inv_n
    mean = jnp.broadcast_to(mean, (c_head, _LANES)).astype(_BF16)
    hid_v[...] = jnp.dot(wdt_v[:, :c_head], mean, preferred_element_type=_F32)

    for h0, nh in last_chunks:
        next(pending).wait()
        xf = rows_v[h0:h0 + nh, head_rows:rpr, :].astype(_F32)
        for g in range(_N_LAST):
            tiles = [xf[h, (g * n_wb + j) * _SUB:(g * n_wb + j + 1) * _SUB, :]
                     for h in range(nh) for j in range(n_wb)]
            acc_last[g] = _tree_sum(tiles + [acc_last[g]])

    m = jnp.sum(jnp.concatenate(acc_last, axis=0), axis=1, keepdims=True) * inv_n
    m = _round_bf16(jnp.broadcast_to(m, (c - c_head, _LANES)))
    terms = [jnp.broadcast_to(m[k:k + 1, :], (r, _LANES)) * wdb_v[k]
             for k in range(c - c_head)]
    terms[0] = terms[0] + hid_v[...]
    half = 0.5 * _round_bf16(_tree_sum(terms))
    hid = _round_bf16(half * jnp.tanh(half) + half)
    hid_b = [jnp.broadcast_to(hid[j:j + 1, :], (_SUB, _LANES)) for j in range(r)]

    def gate(g):
        u_half = _tree_sum(hid_b[j] * wub_v[g, j] for j in range(r))
        return _round_bf16(0.5 * jnp.tanh(_round_bf16(u_half)) + 0.5)

    out_sem = sems.at[0]

    def scale_piece(g, a, b, gates):
        buf[g, a, b] = (buf[g, a, b].astype(_F32) * gates).astype(buf.dtype)

    def piece_gates(p):
        return s_v[pl.ds(p * tpp, tpp)].reshape(piece, _LANES)

    def put_first(a, b, gates):
        scale_piece(0, a, b, gates)
        pltpu.make_async_copy(buf.at[0, a, b], o_hbm.at[0, a, b], out_sem).start()

    first = [gate(g) for g in range(gpp)]
    gates0 = jnp.concatenate([first[t // n_wb] for t in range(tpp)], axis=0)
    for a in range(streams):
        put_first(a, (-a * block) % phases, gates0)

    def warm(p, carry):
        for t in range(gpp * n_wb):
            s_v[t] = first[t // n_wb]
        g0 = jnp.minimum(p, phases - 2) * gpp
        for k in range(gpp):
            s = gate(g0 + k)
            for j in range(n_wb):
                s_v[(g0 + k) * n_wb + j] = s
        gates = piece_gates(p)
        for a in range(streams):
            b = p - (a * block) % phases
            put_first(a, jnp.where(b < 0, b + phases, b), gates)
        return carry

    lax.fori_loop(1, phases, warm, 0)

    def write(i, carry):
        g = i // block
        b = i % block
        p0 = lax.rem(g * (streams * block) + b, phases)
        for a in range(streams):
            p = p0 + (a * block) % phases
            scale_piece(g, a, b, piece_gates(jnp.where(p >= phases, p - phases, p)))
        for k in range(0, piece, _SUB):
            pltpu.make_async_copy(buf.at[g, :, b, pl.ds(k, _SUB)],
                                  o_hbm.at[g, :, b, pl.ds(k, _SUB)], out_sem).start()
        return carry

    lax.fori_loop(phases, groups * block, write, 0)
    pltpu.make_async_copy(buf, o_hbm, out_sem).wait()


@jax.jit
def pallas_standalone__se_block__vision_kernel(
    x: jax.Array,
    w_down: jax.Array,
    w_up: jax.Array,
):
    b, hh, ww, c = x.shape
    assert b == 1
    r = w_down.shape[1]
    n_wb = ww // _LANES
    n_cg = c // _SUB
    rpr = c * n_wb
    rows = x.reshape(hh, n_wb, _LANES, n_cg, _SUB).transpose(0, 3, 1, 4, 2)
    rows = rows.reshape(hh, rpr, _LANES)
    groups = hh * rpr // (_STREAMS * _BLOCK * _PIECE)
    out_shape = (groups, _STREAMS, _BLOCK, _PIECE, _LANES)
    out = pl.pallas_call(
        _se_kernel,
        out_shape=jax.ShapeDtypeStruct(out_shape, x.dtype),
        in_specs=[pl.BlockSpec(memory_space=pl.ANY)] * 3,
        out_specs=pl.BlockSpec(memory_space=pl.ANY),
        scratch_shapes=[
            pltpu.VMEM(out_shape, x.dtype),
            pltpu.VMEM((r, c), w_down.dtype),
            pltpu.VMEM((r, c), w_up.dtype),
            pltpu.VMEM((_N_LAST * _SUB, r, _LANES), _F32),
            pltpu.VMEM((n_cg, r, _SUB, _LANES), _F32),
            pltpu.VMEM((r, _LANES), _F32),
            pltpu.VMEM((rpr // _SUB, _SUB, _LANES), _F32),
            pltpu.SemaphoreType.DMA((_N_READ + 1,)),
        ],
        compiler_params=pltpu.CompilerParams(
            vmem_limit_bytes=100 * 1024 * 1024,
            disable_bounds_checks=True,
            disable_semaphore_checks=True,
        ),
    )(rows, w_down.T, w_up)
    out = out.reshape(hh, n_cg, n_wb, _SUB, _LANES).transpose(0, 2, 4, 1, 3)
    return out.reshape(b, hh, ww, c)
```

```python
import jax
import jax.numpy as jnp
from jax import lax
import jax.experimental.pallas as pl
import jax.experimental.pallas.tpu as pltpu

_LANES = 128
_SUB = 8
_STREAMS = 6
_PIECE = 64
_BLOCK = 64
_BATCH = 16
_N_LAST = 2
_RING = 16
_LAG = 6
_RROWS = 16
_LAST = (16, 5, 2, 1)
_F32 = jnp.float32
_BF16 = jnp.bfloat16


def _split(sizes):
    out, start = [], 0
    for size in sizes:
        out.append((start, size))
        start += size
    return out


def _tree_sum(vals):
    vals = list(vals)
    while len(vals) > 1:
        nxt = [vals[i] + vals[i + 1] for i in range(0, len(vals) - 1, 2)]
        if len(vals) % 2:
            nxt.append(vals[-1])
        vals = nxt
    return vals[0]


def _round_bf16(v):
    return v.astype(_BF16).astype(_F32)


def _divmod_pow2(i, n):
    assert n & (n - 1) == 0
    if isinstance(i, int):
        return divmod(i, n)
    return lax.shift_right_logical(i, n.bit_length() - 1), lax.bitwise_and(i, n - 1)


def _interleave(a, b):
    keyed = [((i + 0.5) / len(a), 1, x) for i, x in enumerate(a)]
    keyed += [((i + 0.5) / len(b), 0, x) for i, x in enumerate(b)]
    return [x for _, _, x in sorted(keyed, key=lambda t: t[:2])]


def _se_kernel(x_hbm, wdt_hbm, wu_hbm, o_hbm,
               buf, wdt_v, wu_v, wdb_v, wub_v, hid_v, s_v, sems):
    n_blocks, block, piece, _ = buf.shape
    r, c = wdt_v.shape
    n_cg = c // _SUB
    n_head = n_cg - _N_LAST
    c_head = n_head * _SUB
    n_tiles = s_v.shape[0] - (_STREAMS - 1) * (piece // _SUB)
    n_wb = n_tiles // n_cg
    tpp = piece // _SUB
    phases = n_tiles // tpp
    keep = piece - _N_LAST * n_wb * _SUB
    gpp = n_cg // (phases - 1)
    inv_n = 1.0 / (n_blocks * block * piece * _LANES // c)
    n_steps = n_blocks // _STREAMS * block
    n_cols = n_blocks // (2 * phases) * block
    n_reg = n_cols - 2 * _LAG
    assert sum(_LAST) == 4 * _LAG and 2 * _LAG < _RING
    assert gpp * (phases - 1) == n_cg and gpp * n_wb >= tpp
    assert block % phases == 1 and block % _BATCH == 0 and phases <= _BATCH
    last_sem = 2 * _RING
    w_sem = last_sem + len(_LAST)

    def column(q, col):
        g, b = _divmod_pow2(col, block)
        return (2 * g + q) * phases, b, sems.at[q * _RING + _divmod_pow2(col, _RING)[1]]

    def region_of(blk0, b, p):
        if isinstance(b, int):
            return blk0 + (p - b) % phases
        a = p - lax.rem(b, phases)
        return blk0 + jnp.where(a < 0, a + phases, a)

    def copy_in(w, sem):
        return pltpu.make_async_copy(x_hbm.at[w], buf.at[w], sem)

    def whole(q, col):
        blk0, b, sem = column(q, col)
        return [(copy_in((pl.ds(blk0, phases), b, pl.ds(k, _RROWS)), sem), q)
                for k in range(0, piece, _RROWS)]

    def partial(q, col):
        blk0, b, sem = column(q, col)
        out = [(copy_in((region_of(blk0, b, p), b), sem), q) for p in range(phases - 1)]
        out.append((copy_in((region_of(blk0, b, phases - 1), b, pl.ds(0, keep)), sem), q))
        return out

    def held_window(f):
        k, q = _divmod_pow2(f, 2)
        blk0, b, _ = column(q, n_reg + k)
        return region_of(blk0, b, phases - 1), b, pl.ds(keep, piece - keep)

    def held(f):
        s = last_sem
        for f0, _ in _split(_LAST)[1:]:
            s = s + (int(f >= f0) if isinstance(f, int) else (f >= f0).astype(jnp.int32))
        return copy_in(held_window(f), sems.at[s])

    def start(copies):
        for cp, q in copies:
            cp.start(priority=q)

    wdt_copy = pltpu.make_async_copy(wdt_hbm, wdt_v, sems.at[w_sem])
    wu_copy = pltpu.make_async_copy(wu_hbm, wu_v, sems.at[w_sem])

    for col in range(_LAG):
        start(whole(1, col))
    wdt_copy.start()
    wu_copy.start()
    for col in range(_LAG):
        start(_interleave(whole(0, col), whole(1, col + _LAG)))

    wdt_copy.wait()
    wu_copy.wait()
    wdt = wdt_v[...].astype(_F32)
    for k in range(c - c_head):
        wdb_v[k] = jnp.broadcast_to(wdt[:, c_head + k:c_head + k + 1], (r, _LANES))
    wut = wu_v[...].astype(_F32).T * 0.5
    for j in range(r):
        col = jnp.broadcast_to(wut[:, j:j + 1], (c, _LANES))
        wub_v[:, j] = col.reshape(n_cg, _SUB, _LANES)

    def add_column(acc, q, col):
        blk0, b, _ = column(q, col)
        row = [buf[region_of(blk0, b, p), b] for p in range(phases - 1)]
        lastp = region_of(blk0, b, phases - 1)
        row.append(buf[lastp, b] if acc.shape[0] == n_cg else buf[lastp, b, 0:keep])
        xf = jnp.concatenate(row, axis=0).astype(_F32)
        xf = xf.reshape(acc.shape[0], n_wb, _SUB, _LANES)
        part = xf[:, 0]
        for j in range(1, n_wb):
            part = part + xf[:, j]
        return acc + part

    def sweep(lo, hi, acc, next0, next1):
        def body(col, acc):
            for q in range(2):
                if acc.shape[0] == n_cg:
                    blk0, b, sem = column(q, col)
                    copy_in((pl.ds(blk0, phases), b), sem).wait()
                else:
                    for cp, _ in partial(q, col):
                        cp.wait()
            if next0 is not None:
                start(_interleave(next0(col + _LAG), next1(col + 2 * _LAG)))
            for q in range(2):
                acc = add_column(acc, q, col)
            return acc
        return lax.fori_loop(lo, hi, body, acc)

    w0, w1 = (lambda col: whole(0, col)), (lambda col: whole(1, col))
    p0, p1 = (lambda col: partial(0, col)), (lambda col: partial(1, col))
    f1 = lambda col: [(held((col - n_cols) * 4 + k), 1) for k in range(4)]
    acc = jnp.zeros((n_cg, _SUB, _LANES), _F32)
    acc = sweep(0, n_reg - 2 * _LAG, acc, w0, w1)
    acc = sweep(n_reg - 2 * _LAG, n_reg - _LAG, acc, w0, p1)
    acc = sweep(n_reg - _LAG, n_reg, acc, p0, p1)
    acc_last = [acc[g] for g in range(n_head, n_cg)]
    acc = acc[:n_head]
    acc = sweep(n_reg, n_reg + _LAG, acc, p0, f1)
    acc = sweep(n_reg + _LAG, n_cols, acc, None, None)

    mean = jnp.sum(acc.reshape(c_head, _LANES), axis=1, keepdims=True) * inv_n
    mean = jnp.broadcast_to(mean, (c_head, _LANES)).astype(_BF16)
    hid_v[...] = jnp.dot(wdt_v[:, :c_head], mean, preferred_element_type=_F32)

    for f0, nf in _split(_LAST):
        for f in range(f0, f0 + nf):
            held(f).wait()
        xf = [buf[held_window(f)].astype(_F32) for f in range(f0, f0 + nf)]
        for g in range(_N_LAST):
            tiles = [v[(g * n_wb + j) * _SUB:(g * n_wb + j + 1) * _SUB, :]
                     for v in xf for j in range(n_wb)]
            acc_last[g] = _tree_sum(tiles + [acc_last[g]])

    m = jnp.sum(jnp.concatenate(acc_last, axis=0), axis=1, keepdims=True) * inv_n
    m = _round_bf16(jnp.broadcast_to(m, (c - c_head, _LANES)))
    terms = [jnp.broadcast_to(m[k:k + 1, :], (r, _LANES)) * wdb_v[k]
             for k in range(c - c_head)]
    terms[0] = terms[0] + hid_v[...]
    half = 0.5 * _round_bf16(_tree_sum(terms))
    hid = _round_bf16(half * jnp.tanh(half) + half)
    hid_b = [jnp.broadcast_to(hid[j:j + 1, :], (_SUB, _LANES)) for j in range(r)]

    def gate(g):
        u_half = _tree_sum(hid_b[j] * wub_v[g, j] for j in range(r))
        return _round_bf16(0.5 * jnp.tanh(_round_bf16(u_half)) + 0.5)

    def scaled(vals, gates):
        return (vals.astype(_F32) * gates.reshape(vals.shape)).astype(vals.dtype)

    def put_piece(a, b, gates):
        buf[a, b] = scaled(buf[a, b], gates)
        pltpu.make_async_copy(buf.at[a, b], o_hbm.at[a, b], sems.at[0]).start()

    first = [gate(g) for g in range(gpp)]
    gates0 = jnp.concatenate([first[t // n_wb] for t in range(tpp)], axis=0)
    for a in range(_STREAMS):
        put_piece(a, -a % phases, gates0)

    def warm(p, carry):
        for t in range(gpp * n_wb):
            s_v[t] = first[t // n_wb]
        g0 = jnp.minimum(p, phases - 2) * gpp
        for k in range(gpp):
            s = gate(g0 + k)
            for j in range(n_wb):
                s_v[(g0 + k) * n_wb + j] = s
        gates = s_v[pl.ds(p * tpp, tpp)]
        for a in range(_STREAMS):
            put_piece(a, jnp.where(p < a, p - a + phases, p - a), gates)
        return carry

    lax.fori_loop(1, phases, warm, 0)
    s_v[n_tiles:] = s_v[0:s_v.shape[0] - n_tiles]

    def wait_batch(n):
        g, b = _divmod_pow2(n * _BATCH, block)
        w = (pl.ds(g * _STREAMS, _STREAMS), pl.ds(b, _BATCH))
        sem = sems.at[_divmod_pow2(n, 2)[1]]
        pltpu.make_async_copy(buf.at[w], o_hbm.at[w], sem).wait()

    def write(i, carry):
        g, b = _divmod_pow2(i, block)
        n, pos = _divmod_pow2(i, _BATCH)
        regions = pl.ds(g * _STREAMS, _STREAMS)
        p = lax.rem(g * _STREAMS + b, phases)
        buf[regions, b] = scaled(buf[regions, b], s_v[pl.ds(p * tpp, _STREAMS * tpp)])
        sem = sems.at[lax.bitwise_and(n, 1)]
        for k in range(0, piece, _SUB):
            w = (regions, b, pl.ds(k, _SUB))
            pltpu.make_async_copy(buf.at[w], o_hbm.at[w], sem).start()

        @pl.when(jnp.logical_and(pos == _BATCH - 1, n > 0))
        def _():
            wait_batch(n - 1)

        return carry

    lax.fori_loop(phases, n_steps, write, 0)
    wait_batch(n_steps // _BATCH - 1)


@jax.jit
def pallas_standalone__se_block__vision_kernel(
    x: jax.Array,
    w_down: jax.Array,
    w_up: jax.Array,
):
    b, hh, ww, c = x.shape
    assert b == 1
    r = w_down.shape[1]
    n_wb = ww // _LANES
    n_cg = c // _SUB
    rpr = c * n_wb
    tiles = x.reshape(hh, n_wb, _LANES, n_cg, _SUB).transpose(0, 3, 1, 4, 2)
    blocks = (hh * rpr // (_BLOCK * _PIECE), _BLOCK, _PIECE, _LANES)
    gate_tiles = (rpr + (_STREAMS - 1) * _PIECE) // _SUB
    out = pl.pallas_call(
        _se_kernel,
        out_shape=jax.ShapeDtypeStruct(blocks, x.dtype),
        in_specs=[pl.BlockSpec(memory_space=pl.ANY)] * 3,
        out_specs=pl.BlockSpec(memory_space=pl.ANY),
        scratch_shapes=[
            pltpu.VMEM(blocks, x.dtype),
            pltpu.VMEM((r, c), w_down.dtype),
            pltpu.VMEM((r, c), w_up.dtype),
            pltpu.VMEM((_N_LAST * _SUB, r, _LANES), _F32),
            pltpu.VMEM((n_cg, r, _SUB, _LANES), _F32),
            pltpu.VMEM((r, _LANES), _F32),
            pltpu.VMEM((gate_tiles, _SUB, _LANES), _F32),
            pltpu.SemaphoreType.DMA((2 * _RING + len(_LAST) + 1,)),
        ],
        compiler_params=pltpu.CompilerParams(
            vmem_limit_bytes=100 * 1024 * 1024,
            disable_bounds_checks=True,
            disable_semaphore_checks=True,
        ),
    )(tiles.reshape(blocks), w_down.T, w_up)
    out = out.reshape(hh, n_cg, n_wb, _SUB, _LANES).transpose(0, 2, 4, 1, 3)
    return out.reshape(b, hh, ww, c)
```

```python
import jax
import jax.numpy as jnp
from jax import lax
import jax.experimental.pallas as pl
import jax.experimental.pallas.tpu as pltpu

_LANES = 128
_SUB = 8
_STREAMS = 6
_PIECE = 64
_BLOCK = 64
_BATCH = 16
_N_LAST = 2
_RING = 16
_RROWS = 8
_SROWS = 16
_GROUP = 2
_LAG = 3
_AHEAD = 6
_LATE = ((10,), (7, 3), (6, 3, 1))
_CUTS = (48, 90)
_PROC = (5, 3)
_F32 = jnp.float32
_BF16 = jnp.bfloat16


def _split(sizes):
    out, start = [], 0
    for size in sizes:
        out.append((start, size))
        start += size
    return out


def _tree_sum(vals):
    vals = list(vals)
    while len(vals) > 1:
        nxt = [vals[i] + vals[i + 1] for i in range(0, len(vals) - 1, 2)]
        if len(vals) % 2:
            nxt.append(vals[-1])
        vals = nxt
    return vals[0]


def _round_bf16(v):
    return v.astype(_BF16).astype(_F32)


def _divmod_pow2(i, n):
    assert n & (n - 1) == 0
    if isinstance(i, int):
        return divmod(i, n)
    return lax.shift_right_logical(i, n.bit_length() - 1), lax.bitwise_and(i, n - 1)


def _interleave(a, b, group):
    runs = -(-min(len(a), len(b)) // group)
    out = []
    for i in range(runs):
        out += b[i * len(b) // runs:(i + 1) * len(b) // runs]
        out += a[i * len(a) // runs:(i + 1) * len(a) // runs]
    return out


def _se_kernel(x_hbm, wdt_hbm, wu_hbm, o_hbm,
               buf, wdt_v, wu_v, wdb_v, wub_v, hid_v, mean_v, s_v, sems):
    n_blocks, block, piece, _ = buf.shape
    r, c = wdt_v.shape
    n_cg = c // _SUB
    n_head = n_cg - _N_LAST
    c_head = n_head * _SUB
    tpp = piece // _SUB
    n_tiles = s_v.shape[0] - (_STREAMS - 1) * tpp
    n_wb = n_tiles // n_cg
    phases = n_tiles // tpp
    keep = piece - _N_LAST * n_wb * _SUB
    p_late = phases - len(_LATE)
    n_early = p_late * tpp // n_wb
    c_early = n_early * _SUB
    gpp = n_cg // (phases - 1)
    inv_n = 1.0 / (n_blocks * block * piece * _LANES // c)
    n_steps = n_blocks // _STREAMS * block
    n_cols = n_blocks // (2 * phases) * block
    n_reg = n_cols - sum(_LATE[0]) // 2
    assert all(sum(sizes) == 2 * (n_cols - n_reg) for sizes in _LATE)
    assert gpp * (phases - 1) == n_cg and gpp * n_wb >= tpp
    assert block % phases == 1 and block % _BATCH == 0 and phases <= _BATCH
    assert _LAG + _AHEAD + n_cols - n_reg <= _RING
    w_sem = 2 * _RING

    def column(q, col):
        g, b = _divmod_pow2(col, block)
        return (2 * g + q) * phases, b, sems.at[q * _RING + _divmod_pow2(col, _RING)[1]]

    def region_of(blk0, b, p):
        if isinstance(b, int):
            return blk0 + (p - b) % phases
        a = p - lax.rem(b, phases)
        return blk0 + jnp.where(a < 0, a + phases, a)

    def copy_in(w, sem):
        return pltpu.make_async_copy(x_hbm.at[w], buf.at[w], sem)

    def whole(q, col, rows=_RROWS, end=piece):
        blk0, b, sem = column(q, col)
        return [(copy_in((pl.ds(blk0, phases), b, pl.ds(k, rows)), sem), q)
                for k in range(0, end, rows)]

    def early(q, col):
        blk0, b, sem = column(q, col)
        a0 = region_of(0, b, 0)
        runs = [(a0, min(p_late, phases - a0)), (0, a0 + p_late - phases)]
        return whole(q, col, end=keep) + [
            (copy_in((pl.ds(blk0 + a, n), b, pl.ds(k, _SROWS)), sem), q)
            for k in range(keep, piece, _SROWS) for a, n in runs if n > 0]

    units = [(q, col) for col in range(n_reg, n_cols) for q in (0, 1)]
    late = []
    for p, sizes in zip(range(p_late, phases), _LATE):
        for u0, nu in _split(sizes):
            sem = sems.at[w_sem + 1 + len(late)]
            wins = []
            for q, col in units[u0:u0 + nu]:
                blk0, b, _ = column(q, col)
                wins.append((region_of(blk0, b, p), b, pl.ds(keep, piece - keep)))
            late.append((p, wins, [copy_in(w, sem) for w in wins]))

    def start(copies):
        for cp, q in copies:
            cp.start(priority=q)

    def cat(lists):
        return [v for lst in lists for v in lst]

    wdt_copy = pltpu.make_async_copy(wdt_hbm, wdt_v, sems.at[w_sem])
    wu_copy = pltpu.make_async_copy(wu_hbm, wu_v, sems.at[w_sem])

    coarse = _RROWS * _AHEAD // _LAG
    start(cat(whole(1, col, coarse) for col in range(_AHEAD)))
    wdt_copy.start()
    wu_copy.start()
    start(_interleave(cat(whole(0, col, coarse) for col in range(_AHEAD)),
                      cat(whole(1, col + _AHEAD) for col in range(_LAG)), 1))

    wdt_copy.wait()
    wu_copy.wait()
    wdt = wdt_v[...].astype(_F32)
    for k in range(c - c_head):
        wdb_v[k] = jnp.broadcast_to(wdt[:, c_head + k:c_head + k + 1], (r, _LANES))
    wut = wu_v[...].astype(_F32).T * 0.5
    for j in range(r):
        col = jnp.broadcast_to(wut[:, j:j + 1], (c, _LANES))
        wub_v[:, j] = col.reshape(n_cg, _SUB, _LANES)

    def add_column(acc, q, col):
        blk0, b, _ = column(q, col)
        row = [buf[region_of(blk0, b, p), b] for p in range(phases)]
        xf = jnp.concatenate(row, axis=0).astype(_F32)
        xf = xf.reshape(n_cg, n_wb, _SUB, _LANES)
        part = xf[:, 0]
        for j in range(1, n_wb):
            part = part + xf[:, j]
        return acc + part

    def sweep(lo, hi, acc, issue):
        def body(col, acc):
            for q in range(2):
                blk0, b, sem = column(q, col)
                copy_in((pl.ds(blk0, phases), b), sem).wait()
            if issue:
                start(_interleave(whole(0, col + _AHEAD),
                                  whole(1, col + _AHEAD + _LAG), _GROUP))
            for q in range(2):
                acc = add_column(acc, q, col)
            return acc
        return lax.fori_loop(lo, hi, body, acc)

    done = n_reg - _AHEAD - _LAG
    acc = sweep(0, done, jnp.zeros((n_cg, _SUB, _LANES), _F32), True)
    rest0 = cat(whole(0, col) for col in range(n_reg - _LAG, n_reg))
    rest0 += cat(early(0, col) for col in range(n_reg, n_cols))
    rest1 = cat(early(1, col) for col in range(n_reg, n_cols))
    rest1 += [(cp, 1) for _, _, copies in late for cp in copies]
    rest = _interleave(rest0, rest1[:len(rest0)], _GROUP) + rest1[len(rest0):]
    cuts = (0,) + _CUTS + (len(rest),)
    for i, n_proc in enumerate(_PROC + (_AHEAD + _LAG - sum(_PROC),)):
        start(rest[cuts[i]:cuts[i + 1]])
        acc = sweep(done, done + n_proc, acc, False)
        done += n_proc

    acc = [acc[g] for g in range(n_cg)]

    def add_rows(parts):
        by_group = {}
        for p, row0, val in parts:
            val = val.astype(_F32)
            for t in range(val.shape[0] // _SUB):
                g = (p * tpp + row0 // _SUB + t) // n_wb
                by_group.setdefault(g, []).append(val[t * _SUB:(t + 1) * _SUB])
        for g, tiles in by_group.items():
            acc[g] = _tree_sum(tiles + [acc[g]])

    def means(g0, g1):
        tot = jnp.sum(jnp.concatenate(acc[g0:g1], axis=0), axis=1, keepdims=True)
        return jnp.broadcast_to(tot * inv_n, ((g1 - g0) * _SUB, _LANES))

    for q, col in units:
        for cp, _ in early(q, col):
            cp.wait()
        blk0, b, _ = column(q, col)
        add_rows([(p, 0, buf[region_of(blk0, b, p), b, 0:piece if p < p_late else keep])
                  for p in range(phases)])
    mean_v[0:c_early] = means(0, n_early).astype(_BF16)
    for i, (p, wins, copies) in enumerate(late):
        if p == phases - 1 and late[i - 1][0] != p:
            mean_v[c_early:c_head] = means(n_early, n_head).astype(_BF16)
        for cp in copies:
            cp.wait()
        add_rows([(p, keep, buf[w]) for w in wins])
        if i == 0:
            hid_v[...] = jnp.dot(wdt_v[:, :c_early], mean_v[0:c_early],
                                 preferred_element_type=_F32)

    m = _round_bf16(means(n_head, n_cg))
    terms = [jnp.broadcast_to(m[k:k + 1, :], (r, _LANES)) * wdb_v[k]
             for k in range(c - c_head)]
    terms[0] = terms[0] + hid_v[...]
    pre = _tree_sum(terms) + jnp.dot(wdt_v[:, c_early:c_head], mean_v[c_early:c_head],
                                     preferred_element_type=_F32)
    half = 0.5 * _round_bf16(pre)
    hid = _round_bf16(half * jnp.tanh(half) + half)
    hid_b = [jnp.broadcast_to(hid[j:j + 1, :], (_SUB, _LANES)) for j in range(r)]

    def gate(g):
        u_half = _tree_sum(hid_b[j] * wub_v[g, j] for j in range(r))
        return _round_bf16(0.5 * jnp.tanh(_round_bf16(u_half)) + 0.5)

    def scaled(vals, gates):
        return (vals.astype(_F32) * gates.reshape(vals.shape)).astype(vals.dtype)

    def put_piece(a, b, gates):
        buf[a, b] = scaled(buf[a, b], gates)
        pltpu.make_async_copy(buf.at[a, b], o_hbm.at[a, b], sems.at[0]).start()

    first = [gate(g) for g in range(gpp)]
    gates0 = jnp.concatenate([first[t // n_wb] for t in range(tpp)], axis=0)
    for a in range(_STREAMS):
        put_piece(a, -a % phases, gates0)

    def warm(p, carry):
        for t in range(gpp * n_wb):
            s_v[t] = first[t // n_wb]
        g0 = jnp.minimum(p, phases - 2) * gpp
        for k in range(gpp):
            s = gate(g0 + k)
            for j in range(n_wb):
                s_v[(g0 + k) * n_wb + j] = s
        gates = s_v[pl.ds(p * tpp, tpp)]
        for a in range(_STREAMS):
            put_piece(a, jnp.where(p < a, p - a + phases, p - a), gates)
        return carry

    lax.fori_loop(1, phases, warm, 0)
    s_v[n_tiles:] = s_v[0:s_v.shape[0] - n_tiles]

    def wait_batch(n):
        g, b = _divmod_pow2(n * _BATCH, block)
        w = (pl.ds(g * _STREAMS, _STREAMS), pl.ds(b, _BATCH))
        sem = sems.at[_divmod_pow2(n, 2)[1]]
        pltpu.make_async_copy(buf.at[w], o_hbm.at[w], sem).wait()

    def write(i, carry):
        g, b = _divmod_pow2(i, block)
        n, pos = _divmod_pow2(i, _BATCH)
        regions = pl.ds(g * _STREAMS, _STREAMS)
        p = lax.rem(g * _STREAMS + b, phases)
        buf[regions, b] = scaled(buf[regions, b], s_v[pl.ds(p * tpp, _STREAMS * tpp)])
        sem = sems.at[lax.bitwise_and(n, 1)]
        for k in range(0, piece, _SUB):
            w = (regions, b, pl.ds(k, _SUB))
            pltpu.make_async_copy(buf.at[w], o_hbm.at[w], sem).start()

        @pl.when(jnp.logical_and(pos == _BATCH - 1, n > 0))
        def _():
            wait_batch(n - 1)

        return carry

    lax.fori_loop(phases, n_steps, write, 0)
    wait_batch(n_steps // _BATCH - 1)


@jax.jit
def pallas_standalone__se_block__vision_kernel(
    x: jax.Array,
    w_down: jax.Array,
    w_up: jax.Array,
):
    b, hh, ww, c = x.shape
    assert b == 1
    r = w_down.shape[1]
    n_wb = ww // _LANES
    n_cg = c // _SUB
    rpr = c * n_wb
    tiles = x.reshape(hh, n_wb, _LANES, n_cg, _SUB).transpose(0, 3, 1, 4, 2)
    blocks = (hh * rpr // (_BLOCK * _PIECE), _BLOCK, _PIECE, _LANES)
    gate_tiles = (rpr + (_STREAMS - 1) * _PIECE) // _SUB
    n_sems = 2 * _RING + 1 + sum(len(sizes) for sizes in _LATE)
    out = pl.pallas_call(
        _se_kernel,
        out_shape=jax.ShapeDtypeStruct(blocks, x.dtype),
        in_specs=[pl.BlockSpec(memory_space=pl.ANY)] * 3,
        out_specs=pl.BlockSpec(memory_space=pl.ANY),
        scratch_shapes=[
            pltpu.VMEM(blocks, x.dtype),
            pltpu.VMEM((r, c), w_down.dtype),
            pltpu.VMEM((r, c), w_up.dtype),
            pltpu.VMEM((_N_LAST * _SUB, r, _LANES), _F32),
            pltpu.VMEM((n_cg, r, _SUB, _LANES), _F32),
            pltpu.VMEM((r, _LANES), _F32),
            pltpu.VMEM((c - _N_LAST * _SUB, _LANES), _BF16),
            pltpu.VMEM((gate_tiles, _SUB, _LANES), _F32),
            pltpu.SemaphoreType.DMA((n_sems,)),
        ],
        compiler_params=pltpu.CompilerParams(
            vmem_limit_bytes=100 * 1024 * 1024,
            disable_bounds_checks=True,
            disable_semaphore_checks=True,
        ),
    )(tiles.reshape(blocks), w_down.T, w_up)
    out = out.reshape(hh, n_cg, n_wb, _SUB, _LANES).transpose(0, 2, 4, 1, 3)
    return out.reshape(b, hh, ww, c)
```

```python
import jax
import jax.numpy as jnp
from jax import lax
import jax.experimental.pallas as pl
import jax.experimental.pallas.tpu as pltpu

_LANES = 128
_SUB = 8
_PIECE = 64
_BLOCK = 64

_WIDTH = 9
_RROWS = 8
_SROWS = 16
_GROUP = 2
_LAG = 3
_AHEAD = 6
_RING = 16
_N_TAIL = 5
_N_LATE = 3
_N_LAST = 2
_TRAIL = ((3,), (4, 1))
_CUTS = (48, 84)
_PROC = (5, 3, 1)

_STREAMS = 6
_BATCH = 16

_F32 = jnp.float32
_BF16 = jnp.bfloat16


def _cat(lists):
    return [v for lst in lists for v in lst]


def _interleave(a, b, group):
    assert len(a) == len(b)
    return _cat(b[i:i + group] + a[i:i + group] for i in range(0, len(a), group))


def _tree_sum(vals):
    vals = list(vals)
    while len(vals) > 1:
        nxt = [vals[i] + vals[i + 1] for i in range(0, len(vals) - 1, 2)]
        if len(vals) % 2:
            nxt.append(vals[-1])
        vals = nxt
    return vals[0]


def _round_bf16(v):
    return v.astype(_BF16).astype(_F32)


def _divmod_pow2(i, n):
    assert n & (n - 1) == 0
    if isinstance(i, int):
        return divmod(i, n)
    return lax.shift_right_logical(i, n.bit_length() - 1), lax.bitwise_and(i, n - 1)


def _se_kernel(x_hbm, wdt_hbm, wu_hbm, o_hbm,
               buf, wdt_v, wu_v, wdb_v, wub_v, acc_v, hid_v, mean_v, s_v, sems):
    n_blocks, block, piece, _ = buf.shape
    r, c = wdt_v.shape
    n_cg = c // _SUB
    n_head = n_cg - _N_LAST
    c_head = n_head * _SUB
    tpp = piece // _SUB
    n_tiles = s_v.shape[0] - (_STREAMS - 1) * tpp
    n_wb = n_tiles // n_cg
    phases = n_tiles // tpp
    keep = piece - _N_LAST * n_wb * _SUB
    p_late = phases - _N_LATE
    n_early = p_late * tpp // n_wb
    c_early = n_early * _SUB
    gpp = n_cg // (phases - 1)
    inv_n = 1.0 / (n_blocks * block * piece * _LANES // c)
    n_cols = n_blocks // (2 * _WIDTH) * block
    n_reg = n_cols - _N_TAIL
    n_steps = n_blocks // _STREAMS * block
    w_sem = 2 * _RING
    assert n_blocks % (2 * _WIDTH) == 0 and n_blocks % _STREAMS == 0
    assert block % phases == 1 and block % _BATCH == 0 and phases <= _BATCH
    assert gpp * (phases - 1) == n_cg and gpp * n_wb >= tpp
    assert sum(_PROC) == _AHEAD + _LAG and _AHEAD + _LAG + _N_TAIL <= _RING

    def column(q, col):
        g, b = _divmod_pow2(col, block)
        sem = sems.at[q * _RING + _divmod_pow2(col, _RING)[1]]
        return (2 * g + q) * _WIDTH, b, sem

    def copy_in(w, sem):
        return pltpu.make_async_copy(x_hbm.at[w], buf.at[w], sem)

    def whole(q, col, rows=_RROWS):
        blk0, b, sem = column(q, col)
        return [(copy_in((pl.ds(blk0, _WIDTH), b, pl.ds(k, rows)), sem), q)
                for k in range(0, piece, rows)]

    def pieces(col):
        blk0, b, _ = column(0, col)
        return [((blk + b) % phases, blk, b) for blk in range(blk0, blk0 + 2 * _WIDTH)]

    def early(half, col):
        blk0, b, _ = column(0, col)
        runs = []
        for p, blk, _ in pieces(col):
            if p < p_late and runs and sum(runs[-1]) == blk:
                runs[-1][1] += 1
            elif p < p_late:
                runs.append([blk, 1])
        wins = [(pl.ds(blk0 + q * _WIDTH, _WIDTH), b, pl.ds(k, _RROWS))
                for k in range(0, keep, _RROWS) for q in range(2)]
        wins += [(pl.ds(blk, n), b, pl.ds(k, _SROWS))
                 for k in range(keep, piece, _SROWS) for blk, n in runs]
        sem = column(half, col)[2]
        return [copy_in(w, sem) for w in wins if w[2].start * 2 // piece == half]

    tail = range(n_reg, n_cols)
    halves = [(half, col) for col in tail for half in range(2)]
    late = []
    for p in range(p_late, phases):
        wins = [(blk, b, pl.ds(keep, piece - keep))
                for col in tail for pos, blk, b in pieces(col) if pos == p]
        if p == phases - 1:
            blk, b, _ = wins.pop()
            cut = piece - n_wb * _SUB
            wins += [(blk, b, pl.ds(keep, cut - keep)), (blk, b, pl.ds(cut, piece - cut))]
        trail = _TRAIL[p - phases] if phases - p <= len(_TRAIL) else ()
        ends = [len(wins) - sum(trail[i:]) for i in range(len(trail) + 1)]
        late += [(p, wins[lo:hi]) for lo, hi in zip([0] + ends[:-1], ends)]
    late = [(p, wins, [copy_in(w, sems.at[w_sem + 1 + i]) for w in wins])
            for i, (p, wins) in enumerate(late)]

    def start(copies):
        for cp, q in copies:
            cp.start(priority=q)

    wdt_copy = pltpu.make_async_copy(wdt_hbm, wdt_v, sems.at[w_sem])
    wu_copy = pltpu.make_async_copy(wu_hbm, wu_v, sems.at[w_sem])

    coarse = _RROWS * _AHEAD // _LAG
    start(_cat(whole(1, col, coarse) for col in range(_AHEAD)))
    wdt_copy.start()
    wu_copy.start()
    start(_interleave(_cat(whole(0, col, coarse) for col in range(_AHEAD)),
                      _cat(whole(1, col + _AHEAD) for col in range(_LAG)), 1))

    acc_v[...] = jnp.zeros(acc_v.shape, _F32)
    wdt_copy.wait()
    wu_copy.wait()
    wdt = wdt_v[...].astype(_F32) * 0.5
    for k in range(c - c_head):
        wdb_v[k] = jnp.broadcast_to(wdt[:, c_head + k:c_head + k + 1], (r, _LANES))
    wut = wu_v[...].astype(_F32).T * 0.5
    for j in range(r):
        wcol = jnp.broadcast_to(wut[:, j:j + 1], (c, _LANES))
        wub_v[:, j] = wcol.reshape(n_cg, _SUB, _LANES)

    def sweep(lo, hi, issue):
        def body(col, carry):
            for q in range(2):
                blk0, b, sem = column(q, col)
                copy_in((pl.ds(blk0, _WIDTH), b), sem).wait()
            if issue:
                start(_interleave(whole(0, col + _AHEAD),
                                  whole(1, col + _AHEAD + _LAG), _GROUP))
            blk0, b, _ = column(0, col)
            xf = buf[pl.ds(blk0, 2 * _WIDTH), b].astype(_F32)
            slots = pl.ds(lax.rem(blk0 + b, phases), phases)
            old = acc_v[slots]
            acc_v[slots] = jnp.stack([
                _tree_sum([old[a]] + [xf[k] for k in range(a, 2 * _WIDTH, phases)])
                for a in range(phases)])
            return carry

        lax.fori_loop(lo, hi, body, 0)

    done = n_reg - _AHEAD - _LAG
    sweep(0, done, True)
    dealt = list(enumerate(_cat(early(*h) for h in halves)))
    rest0 = _cat(whole(0, col) for col in range(n_reg - _LAG, n_reg))
    rest0 += [(cp, 0) for i, cp in dealt if i // _GROUP % 2 == 1]
    rest1 = [(cp, 1) for i, cp in dealt if i // _GROUP % 2 == 0]
    rest1 += [(cp, 1) for _, _, copies in late for cp in copies]
    rest = _interleave(rest0, rest1[:len(rest0)], _GROUP) + rest1[len(rest0):]
    cuts = (0,) + _CUTS + (len(rest),)
    for lo, hi, n_proc in zip(cuts[:-1], cuts[1:], _PROC):
        start(rest[lo:hi])
        sweep(done, done + n_proc, False)
        done += n_proc

    acc = {}

    def add_rows(parts):
        by_group = {}
        for p, row0, val in parts:
            val = val.astype(_F32)
            for t in range(val.shape[0] // _SUB):
                g = (p * tpp + row0 // _SUB + t) // n_wb
                by_group.setdefault(g, []).append(val[t * _SUB:(t + 1) * _SUB])
        for g, tiles in by_group.items():
            acc[g] = _tree_sum(tiles + ([acc[g]] if g in acc else []))

    def means(g0, g1):
        sums = jnp.concatenate([acc[g] for g in range(g0, g1)], axis=0)
        total = jnp.sum(sums, axis=1, keepdims=True)
        return jnp.broadcast_to(total * inv_n, sums.shape)

    add_rows([(k % phases, 0, acc_v[k]) for k in range(acc_v.shape[0])])
    for half, col in halves:
        for cp in early(half, col):
            cp.wait()
        lo, hi = half * piece // 2, (half + 1) * piece // 2
        add_rows([(p, lo, buf[blk, b, lo:hi if p < p_late else keep])
                  for p, blk, b in pieces(col) if p < p_late or lo < keep])
    mean_v[0:c_early] = means(0, n_early).astype(_BF16)
    for i, (p, wins, copies) in enumerate(late):
        if p == phases - 1 and late[i - 1][0] != p:
            mean_v[c_early:c_head] = means(n_early, n_head).astype(_BF16)
        for cp in copies:
            cp.wait()
        if i == 0:
            hid_v[...] = 0.5 * jnp.dot(wdt_v[:, :c_early], mean_v[0:c_early],
                                       preferred_element_type=_F32)
        add_rows([(p, w[2].start, buf[w]) for w in wins])

    m = _round_bf16(means(n_head, n_cg))
    terms = [jnp.broadcast_to(m[k:k + 1, :], (r, _LANES)) * wdb_v[k]
             for k in range(c - c_head)]
    mid = 0.5 * jnp.dot(wdt_v[:, c_early:c_head], mean_v[c_early:c_head],
                        preferred_element_type=_F32)
    before = _tree_sum([hid_v[...]] + terms[:-_SUB]) + mid
    half = _round_bf16(before + _tree_sum(terms[-_SUB:]))
    hid = _round_bf16(half * jnp.tanh(half) + half)
    hid_b = [jnp.broadcast_to(hid[j:j + 1, :], (_SUB, _LANES)) for j in range(r)]

    def gate(g):
        u_half = _tree_sum(hid_b[j] * wub_v[g, j] for j in range(r))
        return _round_bf16(0.5 * jnp.tanh(_round_bf16(u_half)) + 0.5)

    def scaled(vals, gates):
        return (vals.astype(_F32) * gates.reshape(vals.shape)).astype(vals.dtype)

    def put(w, gates):
        buf[w] = scaled(buf[w], gates)
        pltpu.make_async_copy(buf.at[w], o_hbm.at[w], sems.at[0]).start()

    first = [gate(g) for g in range(gpp)]
    edges = [min((g + 1) * n_wb // 2 * 2, tpp) for g in range(gpp)]
    for t0, t1 in zip([0] + edges[:-1], edges):
        gates = jnp.concatenate([first[t // n_wb] for t in range(t0, t1)], axis=0)
        for a in range(_STREAMS):
            put((a, -a % phases, pl.ds(t0 * _SUB, (t1 - t0) * _SUB)), gates)

    def warm(p, carry):
        for t in range(gpp * n_wb):
            s_v[t] = first[t // n_wb]
        g0 = jnp.minimum(p, phases - 2) * gpp
        for k in range(gpp):
            s = gate(g0 + k)
            for j in range(n_wb):
                s_v[(g0 + k) * n_wb + j] = s
        gates = s_v[pl.ds(p * tpp, tpp)]
        for a in range(_STREAMS):
            put((a, jnp.where(p < a, p - a + phases, p - a)), gates)
        return carry

    lax.fori_loop(1, phases, warm, 0)
    s_v[n_tiles:] = s_v[0:s_v.shape[0] - n_tiles]

    def wait_batch(n):
        g, b = _divmod_pow2(n * _BATCH, block)
        w = (pl.ds(g * _STREAMS, _STREAMS), pl.ds(b, _BATCH))
        sem = sems.at[_divmod_pow2(n, 2)[1]]
        pltpu.make_async_copy(buf.at[w], o_hbm.at[w], sem).wait()

    def write(i, carry):
        g, b = _divmod_pow2(i, block)
        n, pos = _divmod_pow2(i, _BATCH)
        regions = pl.ds(g * _STREAMS, _STREAMS)
        p = lax.rem(g * _STREAMS + b, phases)
        buf[regions, b] = scaled(buf[regions, b], s_v[pl.ds(p * tpp, _STREAMS * tpp)])
        sem = sems.at[lax.bitwise_and(n, 1)]
        for k in range(0, piece, _SUB):
            w = (regions, b, pl.ds(k, _SUB))
            pltpu.make_async_copy(buf.at[w], o_hbm.at[w], sem).start()

        @pl.when(jnp.logical_and(pos == _BATCH - 1, n > 0))
        def _():
            wait_batch(n - 1)

        return carry

    lax.fori_loop(phases, n_steps, write, 0)
    wait_batch(n_steps // _BATCH - 1)


@jax.jit
def pallas_standalone__se_block__vision_kernel(
    x: jax.Array,
    w_down: jax.Array,
    w_up: jax.Array,
):
    b, hh, ww, c = x.shape
    assert b == 1
    r = w_down.shape[1]
    n_wb = ww // _LANES
    n_cg = c // _SUB
    rpr = c * n_wb
    tiles = x.reshape(hh, n_wb, _LANES, n_cg, _SUB).transpose(0, 3, 1, 4, 2)
    blocks = (hh * rpr // (_BLOCK * _PIECE), _BLOCK, _PIECE, _LANES)
    gate_tiles = (rpr + (_STREAMS - 1) * _PIECE) // _SUB
    n_sems = 2 * _RING + 1 + _N_LATE + sum(len(t) for t in _TRAIL)
    out = pl.pallas_call(
        _se_kernel,
        out_shape=jax.ShapeDtypeStruct(blocks, x.dtype),
        in_specs=[pl.BlockSpec(memory_space=pl.ANY)] * 3,
        out_specs=pl.BlockSpec(memory_space=pl.ANY),
        scratch_shapes=[
            pltpu.VMEM(blocks, x.dtype),
            pltpu.VMEM((r, c), w_down.dtype),
            pltpu.VMEM((r, c), w_up.dtype),
            pltpu.VMEM((_N_LAST * _SUB, r, _LANES), _F32),
            pltpu.VMEM((n_cg, r, _SUB, _LANES), _F32),
            pltpu.VMEM((2 * rpr // _PIECE - 1, _PIECE, _LANES), _F32),
            pltpu.VMEM((r, _LANES), _F32),
            pltpu.VMEM((c - _N_LAST * _SUB, _LANES), _BF16),
            pltpu.VMEM((gate_tiles, _SUB, _LANES), _F32),
            pltpu.SemaphoreType.DMA((n_sems,)),
        ],
        compiler_params=pltpu.CompilerParams(
            vmem_limit_bytes=100 * 1024 * 1024,
            disable_bounds_checks=True,
            disable_semaphore_checks=True,
        ),
    )(tiles.reshape(blocks), w_down.T, w_up)
    out = out.reshape(hh, n_cg, n_wb, _SUB, _LANES).transpose(0, 2, 4, 1, 3)
    return out.reshape(b, hh, ww, c)
```

```python
import jax
import jax.numpy as jnp
from jax import lax
import jax.experimental.pallas as pl
import jax.experimental.pallas.tpu as pltpu

_LANES = 128
_SUB = 8
_PIECE = 64
_BLOCK = 64

_WIDTHS = ((8, 8), (8, 12), (8, 10))
_RROWS = 8
_SROWS = 16
_GROUP = 2
_LAG = 3
_AHEAD = 6
_RING = 16
_N_TAIL = 7
_N_LATE = 3
_N_LAST = 2
_TRAIL = ((3,), (4, 1))
_CUTS = (48, 96)
_PROC = (5, 3, 1)

_STREAMS = 6
_BATCH = 16

_F32 = jnp.float32
_BF16 = jnp.bfloat16


def _cat(lists):
    return [v for lst in lists for v in lst]


def _interleave(a, b, group):
    assert len(a) == len(b)
    return _cat(b[i:i + group] + a[i:i + group] for i in range(0, len(a), group))


def _tree_sum(vals):
    vals = list(vals)
    while len(vals) > 1:
        nxt = [vals[i] + vals[i + 1] for i in range(0, len(vals) - 1, 2)]
        if len(vals) % 2:
            nxt.append(vals[-1])
        vals = nxt
    return vals[0]


def _round_bf16(v):
    return v.astype(_BF16).astype(_F32)


def _divmod_pow2(i, n):
    assert n & (n - 1) == 0
    if isinstance(i, int):
        return divmod(i, n)
    return lax.shift_right_logical(i, n.bit_length() - 1), lax.bitwise_and(i, n - 1)


def _se_kernel(x_hbm, wdt_hbm, wu_hbm, o_hbm,
               buf, wdt_v, wu_v, wdb_v, wub_v, acc_v, hid_v, mean_v, s_v, sems):
    n_blocks, block, piece, _ = buf.shape
    r, c = wdt_v.shape
    n_cg = c // _SUB
    n_head = n_cg - _N_LAST
    c_head = n_head * _SUB
    tpp = piece // _SUB
    n_tiles = s_v.shape[0] - (_STREAMS - 1) * tpp
    n_wb = n_tiles // n_cg
    phases = n_tiles // tpp
    keep = piece - _N_LAST * n_wb * _SUB
    p_late = phases - _N_LATE
    n_early = p_late * tpp // n_wb
    c_early = n_early * _SUB
    gpp = n_cg // (phases - 1)
    inv_n = 1.0 / (n_blocks * block * piece * _LANES // c)
    n_cols = len(_WIDTHS) * block
    n_reg = n_cols - _N_TAIL
    n_steps = n_blocks // _STREAMS * block
    w_sem = 2 * _RING
    assert sum(map(sum, _WIDTHS)) == n_blocks and n_blocks % _STREAMS == 0
    assert block % phases == 1 and block % _BATCH == 0 and phases <= _BATCH
    assert gpp * (phases - 1) == n_cg and gpp * n_wb >= tpp
    assert sum(_PROC) == _AHEAD + _LAG and _AHEAD + _LAG + _N_TAIL <= _RING

    def column(q, col, like=None):
        g = (col if like is None else like) // block
        first = sum(map(sum, _WIDTHS[:g])) + q * _WIDTHS[g][0]
        sem = sems.at[q * _RING + _divmod_pow2(col, _RING)[1]]
        return pl.ds(first, _WIDTHS[g][q]), col - g * block, sem

    def copy_in(w, sem):
        return pltpu.make_async_copy(x_hbm.at[w], buf.at[w], sem)

    def whole(q, col, like=None):
        regions, b, sem = column(q, col, like)
        return [(copy_in((regions, b, pl.ds(k, _RROWS)), sem), q)
                for k in range(0, piece, _RROWS)]

    def pieces(col):
        regions, b, _ = column(0, col)
        return [((blk + b) % phases, blk, b) for blk in range(regions.start, n_blocks)]

    def early(half, col):
        runs = []
        for p, blk, _ in pieces(col):
            if p < p_late and runs and sum(runs[-1]) == blk:
                runs[-1][1] += 1
            elif p < p_late:
                runs.append([blk, 1])
        _, b, sem = column(half, col)
        wins = [(column(q, col)[0], b, pl.ds(k, _RROWS))
                for k in range(0, keep, _RROWS) for q in range(2)]
        wins += [(pl.ds(blk, n), b, pl.ds(k, _SROWS))
                 for k in range(keep, piece, _SROWS) for blk, n in runs]
        return [copy_in(w, sem) for w in wins if w[2].start * 2 // piece == half]

    tail = range(n_reg, n_cols)
    halves = [(half, col) for col in tail for half in range(2)]
    late = []
    for p in range(p_late, phases):
        wins = [(blk, b, pl.ds(keep, piece - keep))
                for col in tail for pos, blk, b in pieces(col) if pos == p]
        if p == phases - 1:
            blk, b, _ = wins.pop()
            cut = piece - n_wb * _SUB
            wins += [(blk, b, pl.ds(keep, cut - keep)), (blk, b, pl.ds(cut, piece - cut))]
        trail = _TRAIL[p - phases] if phases - p <= len(_TRAIL) else ()
        ends = [len(wins) - sum(trail[i:]) for i in range(len(trail) + 1)]
        late += [(p, wins[lo:hi]) for lo, hi in zip([0] + ends[:-1], ends)]
    late = [(p, wins, [copy_in(w, sems.at[w_sem + 1 + i]) for w in wins])
            for i, (p, wins) in enumerate(late)]

    def start(copies):
        for cp, q in copies:
            cp.start(priority=q)

    wdt_copy = pltpu.make_async_copy(wdt_hbm, wdt_v, sems.at[w_sem])
    wu_copy = pltpu.make_async_copy(wu_hbm, wu_v, sems.at[w_sem])

    start(_cat(whole(1, col) for col in range(_LAG)))
    wdt_copy.start()
    wu_copy.start()
    for col in range(_AHEAD):
        start(_interleave(whole(0, col), whole(1, col + _LAG), _GROUP))

    acc_v[...] = jnp.zeros(acc_v.shape, _F32)
    wdt_copy.wait()
    wu_copy.wait()
    wdt = wdt_v[...].astype(_F32) * 0.5
    for k in range(c - c_head):
        wdb_v[k] = jnp.broadcast_to(wdt[:, c_head + k:c_head + k + 1], (r, _LANES))
    wut = wu_v[...].astype(_F32).T * 0.5
    for j in range(r):
        wcol = jnp.broadcast_to(wut[:, j:j + 1], (c, _LANES))
        wub_v[:, j] = wcol.reshape(n_cg, _SUB, _LANES)

    def add_columns(lo, hi, issue):
        def body(col, carry):
            for q in range(2):
                regions, b, sem = column(q, col, lo)
                copy_in((regions, b), sem).wait()
            if issue:
                k0, k1 = _AHEAD, _AHEAD + _LAG
                start(_interleave(whole(0, col + k0, lo + k0),
                                  whole(1, col + k1, lo + k1), _GROUP))
            regions, b, _ = column(0, col, lo)
            width = sum(_WIDTHS[lo // block])
            xf = buf[pl.ds(regions.start, width), b].astype(_F32)
            slots = pl.ds(lax.rem(regions.start + b, phases), phases)
            old = acc_v[slots]
            acc_v[slots] = jnp.stack([
                _tree_sum([old[a]] + [xf[k] for k in range(a, width, phases)])
                for a in range(phases)])
            return carry

        lax.fori_loop(lo, hi, body, 0)

    done = n_reg - _AHEAD - _LAG
    marks = [0] + [g * block - k for g in range(1, len(_WIDTHS))
                   for k in (_AHEAD + _LAG, _AHEAD, 0)] + [done]
    for lo, hi in zip(marks[:-1], marks[1:]):
        add_columns(lo, hi, True)
    dealt = list(enumerate(_cat(early(*h) for h in halves)))
    rest0 = _cat(whole(0, col) for col in range(n_reg - _LAG, n_reg))
    rest0 += [(cp, 0) for i, cp in dealt if i // _GROUP % 2 == 1]
    rest1 = [(cp, 1) for i, cp in dealt if i // _GROUP % 2 == 0]
    rest1 += [(cp, 1) for _, _, copies in late for cp in copies]
    rest = _interleave(rest0, rest1[:len(rest0)], _GROUP) + rest1[len(rest0):]
    cuts = (0,) + _CUTS + (len(rest),)
    for lo, hi, n_proc in zip(cuts[:-1], cuts[1:], _PROC):
        start(rest[lo:hi])
        add_columns(done, done + n_proc, False)
        done += n_proc

    acc = {}

    def add_rows(parts):
        by_group = {}
        for p, row0, val in parts:
            val = val.astype(_F32)
            for t in range(val.shape[0] // _SUB):
                g = (p * tpp + row0 // _SUB + t) // n_wb
                by_group.setdefault(g, []).append(val[t * _SUB:(t + 1) * _SUB])
        for g, tiles in by_group.items():
            acc[g] = _tree_sum(tiles + ([acc[g]] if g in acc else []))

    def means(g0, g1):
        sums = jnp.concatenate([acc[g] for g in range(g0, g1)], axis=0)
        total = jnp.sum(sums, axis=1, keepdims=True)
        return jnp.broadcast_to(total * inv_n, sums.shape)

    add_rows([(k % phases, 0, acc_v[k]) for k in range(acc_v.shape[0])])
    for half, col in halves:
        for cp in early(half, col):
            cp.wait()
        lo, hi = half * piece // 2, (half + 1) * piece // 2
        add_rows([(p, lo, buf[blk, b, lo:hi if p < p_late else keep])
                  for p, blk, b in pieces(col) if p < p_late or lo < keep])
    mean_v[0:c_early] = means(0, n_early).astype(_BF16)
    for i, (p, wins, copies) in enumerate(late):
        if p == phases - 1 and late[i - 1][0] != p:
            mean_v[c_early:c_head] = means(n_early, n_head).astype(_BF16)
        for cp in copies:
            cp.wait()
        if i == 0:
            hid_v[...] = 0.5 * jnp.dot(wdt_v[:, :c_early], mean_v[0:c_early],
                                       preferred_element_type=_F32)
        add_rows([(p, w[2].start, buf[w]) for w in wins])

    m = _round_bf16(means(n_head, n_cg))
    terms = [jnp.broadcast_to(m[k:k + 1, :], (r, _LANES)) * wdb_v[k]
             for k in range(c - c_head)]
    mid = 0.5 * jnp.dot(wdt_v[:, c_early:c_head], mean_v[c_early:c_head],
                        preferred_element_type=_F32)
    before = _tree_sum([hid_v[...]] + terms[:-_SUB]) + mid
    half = _round_bf16(before + _tree_sum(terms[-_SUB:]))
    hid = _round_bf16(half * jnp.tanh(half) + half)
    hid_b = [jnp.broadcast_to(hid[j:j + 1, :], (_SUB, _LANES)) for j in range(r)]

    def gate(g):
        u_half = _tree_sum(hid_b[j] * wub_v[g, j] for j in range(r))
        return _round_bf16(0.5 * jnp.tanh(_round_bf16(u_half)) + 0.5)

    def scaled(vals, gates):
        return (vals.astype(_F32) * gates.reshape(vals.shape)).astype(vals.dtype)

    def put(w, gates):
        buf[w] = scaled(buf[w], gates)
        pltpu.make_async_copy(buf.at[w], o_hbm.at[w], sems.at[0]).start()

    first = [gate(g) for g in range(gpp)]
    edges = [min((g + 1) * n_wb // 2 * 2, tpp) for g in range(gpp)]
    for t0, t1 in zip([0] + edges[:-1], edges):
        gates = jnp.concatenate([first[t // n_wb] for t in range(t0, t1)], axis=0)
        for a in range(_STREAMS):
            put((a, -a % phases, pl.ds(t0 * _SUB, (t1 - t0) * _SUB)), gates)

    def warm(p, carry):
        for t in range(gpp * n_wb):
            s_v[t] = first[t // n_wb]
        g0 = jnp.minimum(p, phases - 2) * gpp
        for k in range(gpp):
            s = gate(g0 + k)
            for j in range(n_wb):
                s_v[(g0 + k) * n_wb + j] = s
        gates = s_v[pl.ds(p * tpp, tpp)]
        for a in range(_STREAMS):
            put((a, jnp.where(p < a, p - a + phases, p - a)), gates)
        return carry

    lax.fori_loop(1, phases, warm, 0)
    s_v[n_tiles:] = s_v[0:s_v.shape[0] - n_tiles]

    def wait_batch(n):
        g, b = _divmod_pow2(n * _BATCH, block)
        w = (pl.ds(g * _STREAMS, _STREAMS), pl.ds(b, _BATCH))
        sem = sems.at[_divmod_pow2(n, 2)[1]]
        pltpu.make_async_copy(buf.at[w], o_hbm.at[w], sem).wait()

    def write(i, carry):
        g, b = _divmod_pow2(i, block)
        n, pos = _divmod_pow2(i, _BATCH)
        regions = pl.ds(g * _STREAMS, _STREAMS)
        p = lax.rem(g * _STREAMS + b, phases)
        buf[regions, b] = scaled(buf[regions, b], s_v[pl.ds(p * tpp, _STREAMS * tpp)])
        sem = sems.at[lax.bitwise_and(n, 1)]
        for k in range(0, piece, _SUB):
            w = (regions, b, pl.ds(k, _SUB))
            pltpu.make_async_copy(buf.at[w], o_hbm.at[w], sem).start()

        @pl.when(jnp.logical_and(pos == _BATCH - 1, n > 0))
        def _():
            wait_batch(n - 1)

        return carry

    lax.fori_loop(phases, n_steps, write, 0)
    wait_batch(n_steps // _BATCH - 1)


@jax.jit
def pallas_standalone__se_block__vision_kernel(
    x: jax.Array,
    w_down: jax.Array,
    w_up: jax.Array,
):
    b, hh, ww, c = x.shape
    assert b == 1
    r = w_down.shape[1]
    n_wb = ww // _LANES
    n_cg = c // _SUB
    rpr = c * n_wb
    tiles = x.reshape(hh, n_wb, _LANES, n_cg, _SUB).transpose(0, 3, 1, 4, 2)
    blocks = (hh * rpr // (_BLOCK * _PIECE), _BLOCK, _PIECE, _LANES)
    gate_tiles = (rpr + (_STREAMS - 1) * _PIECE) // _SUB
    n_sems = 2 * _RING + 1 + _N_LATE + sum(len(t) for t in _TRAIL)
    out = pl.pallas_call(
        _se_kernel,
        out_shape=jax.ShapeDtypeStruct(blocks, x.dtype),
        in_specs=[pl.BlockSpec(memory_space=pl.ANY)] * 3,
        out_specs=pl.BlockSpec(memory_space=pl.ANY),
        scratch_shapes=[
            pltpu.VMEM(blocks, x.dtype),
            pltpu.VMEM((r, c), w_down.dtype),
            pltpu.VMEM((r, c), w_up.dtype),
            pltpu.VMEM((_N_LAST * _SUB, r, _LANES), _F32),
            pltpu.VMEM((n_cg, r, _SUB, _LANES), _F32),
            pltpu.VMEM((2 * rpr // _PIECE - 1, _PIECE, _LANES), _F32),
            pltpu.VMEM((r, _LANES), _F32),
            pltpu.VMEM((c - _N_LAST * _SUB, _LANES), _BF16),
            pltpu.VMEM((gate_tiles, _SUB, _LANES), _F32),
            pltpu.SemaphoreType.DMA((n_sems,)),
        ],
        compiler_params=pltpu.CompilerParams(
            vmem_limit_bytes=100 * 1024 * 1024,
            disable_bounds_checks=True,
            disable_semaphore_checks=True,
        ),
    )(tiles.reshape(blocks), w_down.T, w_up)
    out = out.reshape(hh, n_cg, n_wb, _SUB, _LANES).transpose(0, 2, 4, 1, 3)
    return out.reshape(b, hh, ww, c)
```
